```python
import os as _os
_os.environ.setdefault("JAX_PLATFORMS", "cpu")
import jax
import jax.numpy as jnp

def _softmax(x, axis=-1):
    return jax.nn.softmax(x, axis=axis)
def _gelu(x):
    return jax.nn.gelu(x, approximate=True)
def _silu(x):
    return jax.nn.silu(x)
def _sigmoid(x):
    return jax.nn.sigmoid(x)
def _layernorm(x, axis=-1, eps=1e-5):
    m = jnp.mean(x, axis=axis, keepdims=True)
    v = jnp.var(x, axis=axis, keepdims=True)
    return (x - m) / jnp.sqrt(v + eps)
def _scatter_add(tgt, idx, src, axis=0):
    return tgt.at[idx].add(src)
def _segment_sum(src, seg, n):
    return jax.ops.segment_sum(src, seg, n)
class _Rng:
    def __init__(self, key):
        self._k = key
    def _next(self):
        self._k, sub = jax.random.split(self._k)
        return sub
    def normal(self, shape):
        return jax.random.normal(self._next(), shape, dtype=jnp.bfloat16)
    def randint(self, lo, hi, shape):
        return jax.random.randint(self._next(), shape, lo, hi, dtype=jnp.int32)
    def uniform(self, shape, lo=0.0, hi=1.0):
        return jax.random.uniform(self._next(), shape, jnp.bfloat16, lo, hi)
    def permutation(self, n):
        return jax.random.permutation(self._next(), n)


kernel_name = 'interleave_layers__gqa_block_cached__dense_activation_silu__decode'

def setup_inputs():
    _rng = _Rng(jax.random.key(int.from_bytes(__import__("os").urandom(4), "little")))
    _w = (lambda a: (lambda t: t.astype(jnp.bfloat16) if jnp.issubdtype(t.dtype, jnp.floating) else t)(jnp.asarray(a)))
    def _A_setup():
        B, Sq, D = 2, 1, 512
        Hq, Hkv, Sk, Dh = 32, 8, 8192, 128
        assert Hq % Hkv == 0, (Hq, Hkv)
        return {
            "x": _w((lambda *s: _rng.normal(s) * 0.1)(B, Sq, D)),
            "k_cache": _w((lambda *s: _rng.normal(s) * 0.8)(B, Hkv, Sk, Dh)),
            "v_cache": _w((lambda *s: _rng.normal(s) * 1.6)(B, Hkv, Sk, Dh)),
            "wq": _w((lambda *s: _rng.normal(s) * 0.8)(D, Hq * Dh) * (D ** -0.5)),
            "wo": _w((lambda *s: _rng.normal(s) * 1.6)(Hq * Dh, D) * ((Hq * Dh) ** -0.5)),
        }
    _A_in = _A_setup()

    def _B_setup():
        B, S, D, F = 2, 1, 512, 1792
        return {
            "x": _w((lambda *s: _rng.normal(s) * 0.1)(B, S, D)),
            "w1": _w((lambda *s: _rng.normal(s) * 0.4)(D, F) * (D ** -0.5)),
            "w2": _w((lambda *s: _rng.normal(s) * 0.4)(F, D) * (F ** -0.5)),
        }
    _B_in = _B_setup()

    return {
        "A_x": _A_in["x"],
        "A_k_cache": _A_in["k_cache"],
        "A_v_cache": _A_in["v_cache"],
        "A_wq": _A_in["wq"],
        "A_wo": _A_in["wo"],
        "B_x": _B_in["x"],
        "B_w1": _B_in["w1"],
        "B_w2": _B_in["w2"],
    }

def reference(A_x, A_k_cache, A_v_cache, A_wq, A_wo, B_x, B_w1, B_w2):
    def _A_ref(x, k_cache, v_cache, wq, wo):
        B, Sq, D = x.shape
        Hq, Dh = 32, 128
        Hkv = k_cache.shape[1]
        rep = Hq // Hkv
        q = (lambda x, *d: x.transpose(*d))((x @ wq).reshape(B, Sq, Hq, Dh), 0, 2, 1, 3)
        k = jnp.repeat(k_cache, rep, axis=1)
        v = jnp.repeat(v_cache, rep, axis=1)
        scores = jnp.einsum("bhqd,bhkd->bhqk", q, k) * (Dh ** -0.5)
        p = _softmax(scores, axis=-1)
        o = jnp.einsum("bhqk,bhkd->bhqd", p, v)
        return (lambda x, *d: x.transpose(*d))(o, 0, 2, 1, 3).reshape(B, Sq, Hq * Dh) @ wo

    def _B_ref(x, w1, w2):
        h = jnp.einsum("bsd,df->bsf", x, w1)
        h = _silu(h)
        out = jnp.einsum("bsf,fd->bsd", h, w2)
        return out

    x = A_x
    x = x + _A_ref(_layernorm(x, axis=-1), A_k_cache, A_v_cache, A_wq, A_wo)
    x = x + _B_ref(_layernorm(x, axis=-1), B_w1, B_w2)
    x = x + _A_ref(_layernorm(x, axis=-1), A_k_cache, A_v_cache, A_wq, A_wo)
    x = x + _B_ref(_layernorm(x, axis=-1), B_w1, B_w2)
    return x
```

```python
import jax
import jax.numpy as jnp
from jax import lax
import jax.experimental.pallas as pl
import jax.experimental.pallas.tpu as pltpu


_REP = 4
_LAST_SPLIT = 4


def _ln(x):
    m = jnp.mean(x, axis=-1, keepdims=True)
    d = x - m
    v = jnp.mean(d * d, axis=-1, keepdims=True)
    return d / jnp.sqrt(v + 1e-5)


def _kernel(x_hbm, k_hbm, v_hbm, wq_hbm, wo_hbm, w1_hbm, w2_hbm, o_ref,
            xs, kb, vb, kt, wq, wo, w1, w2, qs, ksem, vsem, wsem, lsem):
    B, H, S, Dh = kb.shape
    D = xs.shape[-1]
    scale = Dh ** -0.5
    f32, bf16 = jnp.float32, jnp.bfloat16
    ls = S // _LAST_SPLIT

    def w_cp(i):
        src, dst = ((x_hbm, xs), (wq_hbm, wq), (wo_hbm, wo), (w1_hbm, w1),
                    (w2_hbm, w2))[i]
        return pltpu.make_async_copy(src, dst, wsem.at[i])

    def k_cp(b, h):
        return pltpu.make_async_copy(k_hbm.at[b, h], kb.at[b, h], ksem.at[b * H + h])

    def v_cp(b, h):
        return pltpu.make_async_copy(v_hbm.at[b, h], vb.at[b, h], vsem.at[b * H + h])

    def vl_cp(i):
        return pltpu.make_async_copy(v_hbm.at[B - 1, H - 1, pl.ds(i * ls, ls)],
                                     vb.at[B - 1, H - 1, pl.ds(i * ls, ls)],
                                     lsem.at[i])

    for i in range(3):
        w_cp(i).start()
    for h in range(H):
        k_cp(0, h).start()
        v_cp(0, h).start()
    w_cp(3).start()
    w_cp(4).start()
    for h in range(H):
        k_cp(1, h).start()
        if h < H - 1:
            v_cp(1, h).start()
    for i in range(_LAST_SPLIT):
        vl_cp(i).start()

    row = lax.broadcasted_iota(jnp.int32, (8, Dh), 0)

    def make_q(x8, slot):
        q = jnp.dot(_ln(x8).astype(bf16), wq[...], preferred_element_type=f32)
        for h in range(H):
            qh = jnp.zeros((8, Dh), f32)
            for j in range(_REP):
                c = (h * _REP + j) * Dh
                qh = jnp.where(row == j, q[:, c:c + Dh], qh)
            qs[slot, h] = qh

    def softmax_num(s):
        s = s * scale
        m = jnp.max(s, axis=-1, keepdims=True)
        p = jnp.exp(s - m)
        return p.astype(bf16), jnp.sum(p, axis=-1, keepdims=True)

    def qk(q8, b, h):
        return lax.dot_general(q8.astype(bf16), kb[b, h], (((1,), (1,)), ((), ())),
                               preferred_element_type=f32)

    def out_proj(o8, h):
        o = jnp.concatenate(
            [jnp.broadcast_to(o8[j:j + 1], (8, Dh)) for j in range(_REP)], axis=1)
        w = wo[pl.ds(pl.multiple_of(h * _REP * Dh, _REP * Dh), _REP * Dh), :]
        return jnp.dot(o.astype(bf16), w, preferred_element_type=f32)

    def attn_head(slot, b, h, wait, transpose=False):
        if wait:
            k_cp(b, h).wait()
        if transpose:
            kt[h] = kb[b, h].T
        p, l = softmax_num(qk(qs[slot, h], b, h))
        if wait:
            v_cp(b, h).wait()
        o8 = jnp.dot(p, vb[b, h], preferred_element_type=f32) / l
        return out_proj(o8, h)

    def ffn(x8):
        hdn = jnp.dot(_ln(x8).astype(bf16), w1[...], preferred_element_type=f32)
        hdn = hdn * jax.nn.sigmoid(hdn)
        return x8 + jnp.dot(hdn.astype(bf16), w2[...], preferred_element_type=f32)

    w_cp(0).wait()
    x = xs[...].astype(f32)
    x0 = jnp.broadcast_to(x[0:1], (8, D))
    x1 = jnp.broadcast_to(x[1:2], (8, D))
    w_cp(1).wait()
    make_q(x0, 0)
    make_q(x1, 1)
    w_cp(2).wait()

    x0 = lax.fori_loop(0, H, lambda h, a: a + attn_head(0, 0, h, True), x0)
    w_cp(3).wait()
    w_cp(4).wait()
    x0 = ffn(x0)
    make_q(x0, 0)

    def both(h, c):
        a0, a1 = c
        a0 = a0 + attn_head(0, 0, h, False)
        a1 = a1 + attn_head(1, 1, h, True, transpose=True)
        return a0, a1

    x0, x1 = lax.fori_loop(0, H - 1, both, (x0, x1))
    x0 = x0 + attn_head(0, 0, H - 1, False)
    x0 = ffn(x0)
    o_ref[0:1, :] = x0[0:1].astype(o_ref.dtype)

    h = H - 1
    k_cp(1, h).wait()
    kt[h] = kb[1, h].T
    p, l = softmax_num(qk(qs[1, h], 1, h))
    o8 = jnp.zeros((8, Dh), f32)
    for i in range(_LAST_SPLIT):
        vl_cp(i).wait()
        o8 = o8 + jnp.dot(p[:, i * ls:(i + 1) * ls], vb[1, h, pl.ds(i * ls, ls), :],
                          preferred_element_type=f32)
    x1 = x1 + out_proj(o8 / l, h)

    x1 = ffn(x1)
    make_q(x1, 1)

    def tail(h, a):
        s = jnp.dot(qs[1, h].astype(bf16), kt[h], preferred_element_type=f32)
        p, l = softmax_num(s)
        o8 = jnp.dot(p, vb[1, h], preferred_element_type=f32) / l
        return a + out_proj(o8, h)

    x1 = lax.fori_loop(0, H, tail, x1)
    x1 = ffn(x1)
    o_ref[1:2, :] = x1[0:1].astype(o_ref.dtype)


@jax.jit
def pallas_interleave_layers__gqa_block_cached__dense_activation_silu__decode_kernel(
    A_x: jax.Array,
    A_k_cache: jax.Array,
    A_v_cache: jax.Array,
    A_wq: jax.Array,
    A_wo: jax.Array,
    B_x: jax.Array,
    B_w1: jax.Array,
    B_w2: jax.Array,
):
    del B_x
    B, Sq, D = A_x.shape
    _, H, S, Dh = A_k_cache.shape
    dt = A_k_cache.dtype
    out = pl.pallas_call(
        _kernel,
        out_shape=jax.ShapeDtypeStruct((B, D), A_x.dtype),
        in_specs=[pl.BlockSpec(memory_space=pl.ANY)] * 7,
        out_specs=pl.BlockSpec(memory_space=pltpu.VMEM),
        scratch_shapes=[
            pltpu.VMEM((B, D), A_x.dtype),
            pltpu.VMEM((B, H, S, Dh), dt),
            pltpu.VMEM((B, H, S, Dh), dt),
            pltpu.VMEM((H, Dh, S), dt),
            pltpu.VMEM(A_wq.shape, A_wq.dtype),
            pltpu.VMEM(A_wo.shape, A_wo.dtype),
            pltpu.VMEM(B_w1.shape, B_w1.dtype),
            pltpu.VMEM(B_w2.shape, B_w2.dtype),
            pltpu.VMEM((B, H, 8, Dh), jnp.float32),
            pltpu.SemaphoreType.DMA((B * H,)),
            pltpu.SemaphoreType.DMA((B * H,)),
            pltpu.SemaphoreType.DMA((5,)),
            pltpu.SemaphoreType.DMA((_LAST_SPLIT,)),
        ],
        compiler_params=pltpu.CompilerParams(vmem_limit_bytes=120 * 1024 * 1024),
    )(A_x.reshape(B, D), A_k_cache, A_v_cache, A_wq, A_wo, B_w1, B_w2)
    return out.reshape(B, Sq, D)
```

```python
import functools

import jax
import jax.numpy as jnp
from jax import lax
import jax.experimental.pallas as pl
import jax.experimental.pallas.tpu as pltpu


_NKV = 4
_NV = 3
_LEAD, _TRAIL = 1, 4
_REP = 4
_GROUPS = ((0, 0, 4), (0, 4, 4), (1, 0, 4), (1, 4, 2), (1, 6, 1), (1, 7, 1))
_LAST = ((0, 4096), (4096, 3072), (7168, 1024))


def _ln(x):
    m = jnp.mean(x, axis=-1, keepdims=True)
    d = x - m
    v = jnp.mean(d * d, axis=-1, keepdims=True)
    return d / jnp.sqrt(v + 1e-5)


def _kernel(x_hbm, k_hbm, v_hbm, wq_hbm, wo_hbm, w1_hbm, w2_hbm, o_ref,
            xs, kb, vb, kt, wq, wo, w1, w2, wqt, wot, w1t, w2t, ycol, ocol, hcol,
            cs1, csq, ktf, qcol, qs, ksem, vsem, wsem, lsem):
    B, H, S, Dh = kb.shape
    D = xs.shape[-1]
    scale = Dh ** -0.5
    f32, bf16 = jnp.float32, jnp.bfloat16

    def w_cp(i):
        src, dst = ((x_hbm, xs), (wq_hbm, wq), (wo_hbm, wo), (w1_hbm, w1),
                    (w2_hbm, w2))[i]
        return pltpu.make_async_copy(src, dst, wsem.at[i])

    def kv_cp(t, g):
        b, h0, n = _GROUPS[g]
        src, dst, sem = ((k_hbm, kb, ksem), (v_hbm, vb, vsem))[t]
        return pltpu.make_async_copy(src.at[b, pl.ds(h0, n)], dst.at[b, pl.ds(h0, n)],
                                     sem.at[g])

    def vl_cp(i):
        r0, n = _LAST[i]
        return pltpu.make_async_copy(v_hbm.at[B - 1, H - 1, pl.ds(r0, n)],
                                     vb.at[B - 1, H - 1, pl.ds(r0, n)], lsem.at[i])

    G = len(_GROUPS)
    queue = [w_cp(i) for i in range(5)]
    for g in range(G - 1):
        queue += [kv_cp(0, g), kv_cp(1, g)]
    queue += [kv_cp(0, G - 1)] + [vl_cp(i) for i in range(len(_LAST))]

    def enqueue(i, c):
        for j, cp in enumerate(queue):
            pl.when(i == j)(cp.start)
        return c

    lax.fori_loop(0, len(queue), enqueue, 0)

    def kv_wait(t, b, h):
        for g, (gb, h0, _) in enumerate(_GROUPS[:-1]):
            if gb == b:
                pl.when(h == h0)(kv_cp(t, g).wait)

    row = lax.broadcasted_iota(jnp.int32, (8, Dh), 0)

    def make_q(x8, slot):
        q = jnp.dot(_ln(x8).astype(bf16), wq[...], preferred_element_type=f32)
        for h in range(H):
            qh = jnp.zeros((8, Dh), f32)
            for j in range(_REP):
                c = (h * _REP + j) * Dh
                qh = jnp.where(row == j, q[:, c:c + Dh], qh)
            qs[slot, h] = qh

    def softmax_num(s):
        s = s * scale
        m = jnp.max(s, axis=-1, keepdims=True)
        p = jnp.exp(s - m)
        return p.astype(bf16), jnp.sum(p, axis=-1, keepdims=True)

    def qk(q8, b, h):
        return lax.dot_general(q8.astype(bf16), kb[b, h], (((1,), (1,)), ((), ())),
                               preferred_element_type=f32)

    def out_proj(o8, h):
        o = jnp.concatenate(
            [jnp.broadcast_to(o8[j:j + 1], (8, Dh)) for j in range(_REP)], axis=1)
        r0 = h * _REP * Dh
        w = wo[pl.ds(r0 if isinstance(h, int) else pl.multiple_of(r0, _REP * Dh), _REP * Dh), :]
        return jnp.dot(o.astype(bf16), w, preferred_element_type=f32)

    def transpose_k(h):
        for t in range(S // Dh):
            tile = kb[1, h, t * Dh:(t + 1) * Dh, :].T
            kt[h, t] = tile
            if t >= S // Dh - _NKV:
                ktf[h, t - (S // Dh - _NKV)] = tile.astype(f32)

    def attn_head(slot, b, h, wait, transpose=False):
        if wait:
            kv_wait(0, b, h)
        if transpose:
            transpose_k(h)
        p, l = softmax_num(qk(qs[slot, h], b, h))
        if wait:
            kv_wait(1, b, h)
        o8 = jnp.dot(p, vb[b, h], preferred_element_type=f32) / l
        return out_proj(o8, h)

    def ffn(x8):
        hdn = jnp.dot(_ln(x8).astype(bf16), w1[...], preferred_element_type=f32)
        hdn = hdn * jax.nn.sigmoid(hdn)
        return x8 + jnp.dot(hdn.astype(bf16), w2[...], preferred_element_type=f32)

    w_cp(0).wait()
    x = xs[...].astype(f32)
    x0 = jnp.broadcast_to(x[0:1], (8, D))
    x1 = jnp.broadcast_to(x[1:2], (8, D))
    w_cp(1).wait()
    make_q(x0, 0)
    make_q(x1, 1)
    w_cp(2).wait()

    for j in range(wqt.shape[0]):
        wqt[j] = wq[:, j * Dh:(j + 1) * Dh].astype(wqt.dtype)
    for j in range(wot.shape[0]):
        wot[j] = wo[:, j * Dh:(j + 1) * Dh].astype(wot.dtype)

    x0 = lax.fori_loop(0, H, lambda h, a: a + attn_head(0, 0, h, True), x0)
    w_cp(3).wait()
    w_cp(4).wait()
    x0 = ffn(x0)
    make_q(x0, 0)
    for j in range(w1t.shape[0]):
        w = w1[:, j * Dh:(j + 1) * Dh]
        w1t[j] = w
        cs1[j] = jnp.broadcast_to(jnp.sum(w.astype(f32), axis=0, keepdims=True), (8, Dh))
    for j in range(w2t.shape[0]):
        w2t[j] = w2[:, j * Dh:(j + 1) * Dh]

    def colsum_q(h, c):
        cs = jnp.zeros((8, Dh), f32)
        for j in range(_REP):
            t = jnp.sum(wqt[h * _REP + j].astype(f32), axis=0, keepdims=True)
            cs = jnp.where(row == j, t, cs)
        csq[h] = cs
        return c

    lax.fori_loop(0, H, colsum_q, 0)

    x0 = lax.fori_loop(0, H, lambda h, a: a + attn_head(0, 0, h, False), x0)
    x0 = ffn(x0)
    o_ref[0:1, :] = x0[0:1].astype(o_ref.dtype)

    x1 = lax.fori_loop(
        0, H - 1, lambda h, a: a + attn_head(1, 1, h, True, transpose=True), x1)
    h = H - 1
    kv_cp(0, G - 1).wait()
    transpose_k(h)
    p, l = softmax_num(qk(qs[1, h], 1, h))
    o8 = jnp.zeros((8, Dh), f32)
    for i, (r0, n) in enumerate(_LAST):
        vl_cp(i).wait()
        o8 = o8 + jnp.dot(p[:, r0:r0 + n], vb[1, h, r0:r0 + n, :],
                          preferred_element_type=f32)
    x1 = x1 + out_proj(o8 / l, h)

    true = (pltpu.bitcast(x1[:, :Dh], jnp.int32) | 1) != 0

    def after(val, dep):
        return val if dep is None else jnp.where(true, val, dep)

    def col(v):
        return jnp.broadcast_to(v, (Dh, Dh)).T

    def vpu_rows(acc, w_ref, tiles, row0, c_ref, c0, dep):
        cl = after(c_ref[c0:c0 + 8, :], dep)
        ch = after(c_ref[c0 + 8:c0 + 16, :], dep)
        for j, t in enumerate(tiles):
            w = w_ref[t, row0:row0 + 16, :].astype(f32)
            u = w[:8] * cl + w[8:] * ch
            acc[j] = u if acc[j] is None else acc[j] + u

    def ld(ref32, idx, r0, n):
        return pltpu.bitcast(ref32[idx + (slice(r0 // 2, (r0 + n) // 2),)], bf16)

    def ln_parts(x8):
        xb = x8.astype(bf16)
        xr = xb.astype(f32)
        for i in range(D // Dh):
            ycol[i * Dh:(i + 1) * Dh, :] = col(xr[0:1, i * Dh:(i + 1) * Dh])
        m = jnp.mean(xr, axis=-1, keepdims=True)
        d = xr - m
        v = jnp.mean(d * d, axis=-1, keepdims=True)
        return xb, m, 1.0 / jnp.sqrt(v + 1e-5)

    w1t32, w2t32 = w1t.bitcast(jnp.uint32), w2t.bitcast(jnp.uint32)
    NF = w1t.shape[0]
    NV = _NV
    NM = NF - NV

    def gated(n, deps):
        deps = [None] * _LEAD + deps[:len(deps) - _TRAIL]
        return [deps[i * len(deps) // n] for i in range(n)]

    def ffn_tail(x8):
        xb, m, r = ln_parts(x8)

        def act(u, n):
            z = (u - m * cs1[n]) * r
            return z * jax.nn.sigmoid(z)

        us = [jnp.dot(xb, ld(w1t32, (n,), 0, D), preferred_element_type=f32)
              for n in range(NM)]
        hs = [act(u, n) for n, u in enumerate(us)]
        for n in range(NV):
            hcol[n * Dh:(n + 1) * Dh, :] = col(hs[n][0:1])
        acc = [None] * NV
        for i, dep in enumerate(gated(D // 16, us)):
            vpu_rows(acc, w1t, range(NM, NF), i * 16, ycol, i * 16, dep)
        hs += [act(jnp.sum(a, axis=0, keepdims=True), NM + j)
               for j, a in enumerate(acc)]
        ds = []
        for k in range(NV, NF):
            w = jnp.concatenate([ld(w2t32, (n,), k * Dh, Dh) for n in range(D // Dh)],
                                axis=1)
            ds.append(jnp.dot(hs[k].astype(bf16), w, preferred_element_type=f32))
        acc = [None] * (D // Dh)
        for i, dep in enumerate(gated(NV * Dh // 16, [d[:, :Dh] for d in ds])):
            vpu_rows(acc, w2t, range(D // Dh), i * 16, hcol, i * 16, dep)
        out = x8 + jnp.concatenate(
            [jnp.sum(a, axis=0, keepdims=True) for a in acc], axis=1)
        for d in ds:
            out = out + d
        return out

    x1 = ffn_tail(x1)
    xb, m2, r2 = ln_parts(x1)
    q0 = jnp.dot(xb, wq[:, :_REP * Dh], preferred_element_type=f32)
    q8 = jnp.zeros((8, Dh), f32)
    for j in range(_REP):
        q8 = jnp.where(row == j, q0[:, j * Dh:(j + 1) * Dh], q8)
    qrow = {0: (q8 - m2 * csq[0]) * r2}

    vb32 = vb.bitcast(jnp.uint32)
    kt32 = kt.bitcast(jnp.uint32)
    NT = S // Dh
    oacc = [None] * (D // Dh)

    def fold4(a):
        def mix(u, v, sh):
            m = (row & sh) == 0
            return jnp.where(m, u, v) + pltpu.roll(jnp.where(m, v, u), sh, 0)
        c = mix(mix(a[0], a[1], 1), mix(a[2], a[3], 1), 2)
        return c + pltpu.roll(c, 4, 0)

    def wq_work(h):
        acc = [None] * _REP

        def chunk(r, dep):
            vpu_rows(acc, wqt, range(h * _REP, (h + 1) * _REP), r * 16, ycol, r * 16, dep)
            if r == D // 16 - 1:
                qrow[h] = (fold4(acc) - m2 * csq[h]) * r2
                for j in range(_REP):
                    qcol[h, j * Dh:(j + 1) * Dh, :] = col(qrow[h][j:j + 1])
        return [functools.partial(chunk, r) for r in range(D // 16)]

    def wo_work(h):
        def chunk(r, dep):
            vpu_rows(oacc, wot, range(D // Dh), h * _REP * Dh + r * 16,
                     ocol.at[h % 2], r * 16, dep)
        return [functools.partial(chunk, r) for r in range(_REP * Dh // 16)]

    def qk_work(h, out):
        work = []
        for t0 in range(0, _NKV, 4):
            acc = [[None] * _REP for _ in range(4)]

            def chunk(g, dep, t0=t0, acc=acc):
                qv = [after(qcol[h, j * Dh + g * 8:j * Dh + g * 8 + 8, :], dep)
                      for j in range(_REP)]
                for t in range(4):
                    kv = ktf[h, t0 + t, g * 8:g * 8 + 8, :]
                    for j in range(_REP):
                        u = kv * qv[j]
                        acc[t][j] = u if g == 0 else acc[t][j] + u
                if g == Dh // 8 - 1:
                    out.extend(fold4(a) for a in acc)
            work += [functools.partial(chunk, g) for g in range(Dh // 8)]
        return work

    def run(steps, work):
        res = []
        for i, step in enumerate(steps):
            res.append(step())
            for w in work[i * len(work) // len(steps):(i + 1) * len(work) // len(steps)]:
                w(res[i - 1][:, :Dh] if i else None)
        return res

    def qk_stage(h):
        qb = qrow[h].astype(bf16)

        def step(t0):
            kk = jnp.concatenate([ld(kt32, (h, t0 + t), 0, Dh) for t in range(4)], axis=1)
            return jnp.dot(qb, kk, preferred_element_type=f32)
        extra = []
        work = qk_work(h, extra) if h else wq_work(1) + wq_work(2)
        ss = run([functools.partial(step, t0)
                  for t0 in range(0, NT - (_NKV if h else 0), 4)], work)
        return jnp.concatenate(ss + extra, axis=1)

    def pv_stage(h, s):
        p, l = softmax_num(s)
        cs = 4 * Dh

        def step(c0):
            return jnp.dot(p[:, c0:c0 + cs], ld(vb32, (1, h), c0, cs),
                           preferred_element_type=f32)
        work = (wq_work(h + 3) if h + 3 < H else []) + (wo_work(h - 1) if h else [])
        ds = run([functools.partial(step, c0) for c0 in range(0, S, cs)], work)
        o8 = functools.reduce(lambda a, b: a + b, ds) / l
        if h + 1 < H:
            for j in range(_REP):
                ocol[h % 2, j * Dh:(j + 1) * Dh, :] = col(o8[j:j + 1])
        return o8

    s_prev = qk_stage(0)
    for h in range(H):
        if h + 1 < H:
            s_next = qk_stage(h + 1)
        o8 = pv_stage(h, s_prev)
        s_prev = s_next
    x1 = x1 + out_proj(o8, H - 1) + jnp.concatenate(
        [jnp.sum(a, axis=0, keepdims=True) for a in oacc], axis=1)
    x1 = ffn_tail(x1)
    o_ref[1:2, :] = x1[0:1].astype(o_ref.dtype)


@jax.jit
def pallas_interleave_layers__gqa_block_cached__dense_activation_silu__decode_kernel(
    A_x: jax.Array,
    A_k_cache: jax.Array,
    A_v_cache: jax.Array,
    A_wq: jax.Array,
    A_wo: jax.Array,
    B_x: jax.Array,
    B_w1: jax.Array,
    B_w2: jax.Array,
):
    del B_x
    B, Sq, D = A_x.shape
    _, H, S, Dh = A_k_cache.shape
    F = B_w1.shape[1]
    dt = A_k_cache.dtype
    out = pl.pallas_call(
        _kernel,
        out_shape=jax.ShapeDtypeStruct((B, D), A_x.dtype),
        in_specs=[pl.BlockSpec(memory_space=pl.ANY)] * 7,
        out_specs=pl.BlockSpec(memory_space=pltpu.VMEM),
        scratch_shapes=[
            pltpu.VMEM((B, D), A_x.dtype),
            pltpu.VMEM((B, H, S, Dh), dt),
            pltpu.VMEM((B, H, S, Dh), dt),
            pltpu.VMEM((H, S // Dh, Dh, Dh), dt),
            pltpu.VMEM(A_wq.shape, A_wq.dtype),
            pltpu.VMEM(A_wo.shape, A_wo.dtype),
            pltpu.VMEM(B_w1.shape, B_w1.dtype),
            pltpu.VMEM(B_w2.shape, B_w2.dtype),
            pltpu.VMEM((A_wq.shape[1] // Dh, D, Dh), jnp.float32),
            pltpu.VMEM((D // Dh, A_wo.shape[0], Dh), jnp.float32),
            pltpu.VMEM((F // Dh, D, Dh), B_w1.dtype),
            pltpu.VMEM((D // Dh, F, Dh), B_w2.dtype),
            pltpu.VMEM((D, Dh), jnp.float32),
            pltpu.VMEM((2, _REP * Dh, Dh), jnp.float32),
            pltpu.VMEM((_NV * Dh, Dh), jnp.float32),
            pltpu.VMEM((F // Dh, 8, Dh), jnp.float32),
            pltpu.VMEM((H, 8, Dh), jnp.float32),
            pltpu.VMEM((H, _NKV, Dh, Dh), jnp.float32),
            pltpu.VMEM((H, _REP * Dh, Dh), jnp.float32),
            pltpu.VMEM((B, H, 8, Dh), jnp.float32),
            pltpu.SemaphoreType.DMA((len(_GROUPS),)),
            pltpu.SemaphoreType.DMA((len(_GROUPS) - 1,)),
            pltpu.SemaphoreType.DMA((5,)),
            pltpu.SemaphoreType.DMA((len(_LAST),)),
        ],
        compiler_params=pltpu.CompilerParams(vmem_limit_bytes=126 * 1024 * 1024),
    )(A_x.reshape(B, D), A_k_cache, A_v_cache, A_wq, A_wo, B_w1, B_w2)
    return out.reshape(B, Sq, D)
```

```python
import functools

import jax
import jax.numpy as jnp
from jax import lax
import jax.experimental.pallas as pl
import jax.experimental.pallas.tpu as pltpu


_NKV = 4
_NV = 3
_LEAD, _TRAIL = 2, 5
_REP = 4
_GROUPS = ((0, 0, 8), (1, 0, 4), (1, 4, 2), (1, 6, 1), (1, 7, 1))
_LAST = ((0, 4096), (4096, 2560), (6656, 1024), (7680, 512))


def _ln(x):
    m = jnp.mean(x, axis=-1, keepdims=True)
    d = x - m
    v = jnp.mean(d * d, axis=-1, keepdims=True)
    return d / jnp.sqrt(v + 1e-5)


def _kernel(x_hbm, k_hbm, v_hbm, wq_hbm, wo_hbm, w1_hbm, w2_hbm, o_ref,
            xs, kb, vb, kt, wq, wo, w1, w2, wqt, wot, w1t, w2t, ycol, ocol, hcol,
            cs1, csq, ktf, qcol, qs, ksem, vsem, wsem, lsem):
    B, H, S, Dh = kb.shape
    D = xs.shape[-1]
    scale = Dh ** -0.5
    f32, bf16 = jnp.float32, jnp.bfloat16

    def w_cp(i):
        src, dst = ((x_hbm, xs), (wq_hbm, wq), (wo_hbm, wo), (w1_hbm, w1),
                    (w2_hbm, w2))[i]
        return pltpu.make_async_copy(src, dst, wsem.at[i])

    def kv_cp(t, g):
        b, h0, n = _GROUPS[g]
        src, dst, sem = ((k_hbm, kb, ksem), (v_hbm, vb, vsem))[t]
        return pltpu.make_async_copy(src.at[b, pl.ds(h0, n)], dst.at[b, pl.ds(h0, n)],
                                     sem.at[g])

    def vl_cp(i):
        r0, n = _LAST[i]
        return pltpu.make_async_copy(v_hbm.at[B - 1, H - 1, pl.ds(r0, n)],
                                     vb.at[B - 1, H - 1, pl.ds(r0, n)], lsem.at[i])

    G = len(_GROUPS)
    w_cp(1).start()
    queue = [w_cp(i) for i in (0, 2, 3, 4)]
    for g in range(G - 2):
        queue += [kv_cp(0, g), kv_cp(1, g)]
    queue += [kv_cp(0, G - 2), kv_cp(0, G - 1), kv_cp(1, G - 2)]
    queue += [vl_cp(i) for i in range(len(_LAST))]

    def enqueue(i, c):
        for j, cp in enumerate(queue):
            pl.when(i == j)(cp.start)
        return c

    lax.fori_loop(0, len(queue), enqueue, 0)

    def kv_wait(t, b, h):
        for g, (gb, h0, _) in enumerate(_GROUPS[:-2]):
            if gb == b:
                pl.when(h == h0)(kv_cp(t, g).wait)

    row = lax.broadcasted_iota(jnp.int32, (8, Dh), 0)

    def make_q(x8, slot):
        q = jnp.dot(_ln(x8).astype(bf16), wq[...], preferred_element_type=f32)
        for h in range(H):
            qh = jnp.zeros((8, Dh), f32)
            for j in range(_REP):
                c = (h * _REP + j) * Dh
                qh = jnp.where(row == j, q[:, c:c + Dh], qh)
            qs[slot, h] = qh

    def softmax_num(s):
        s = s * scale
        m = jnp.max(s, axis=-1, keepdims=True)
        p = jnp.exp(s - m)
        return p.astype(bf16), jnp.sum(p, axis=-1, keepdims=True)

    def qk(q8, b, h):
        return lax.dot_general(q8.astype(bf16), kb[b, h], (((1,), (1,)), ((), ())),
                               preferred_element_type=f32)

    def out_proj(o8, h):
        o = jnp.concatenate(
            [jnp.broadcast_to(o8[j:j + 1], (8, Dh)) for j in range(_REP)], axis=1)
        r0 = h * _REP * Dh
        w = wo[pl.ds(r0 if isinstance(h, int) else pl.multiple_of(r0, _REP * Dh), _REP * Dh), :]
        return jnp.dot(o.astype(bf16), w, preferred_element_type=f32)

    def transpose_k(h):
        for t in range(S // Dh):
            tile = kb[1, h, t * Dh:(t + 1) * Dh, :].T
            kt[h, t] = tile
            if t >= S // Dh - _NKV:
                ktf[h, t - (S // Dh - _NKV)] = tile.astype(f32)

    def attn_head(slot, b, h, wait, transpose=False):
        if wait:
            kv_wait(0, b, h)
        if transpose:
            transpose_k(h)
        p, l = softmax_num(qk(qs[slot, h], b, h))
        if wait:
            kv_wait(1, b, h)
        o8 = jnp.dot(p, vb[b, h], preferred_element_type=f32) / l
        return out_proj(o8, h)

    def ffn(x8):
        hdn = jnp.dot(_ln(x8).astype(bf16), w1[...], preferred_element_type=f32)
        hdn = hdn * jax.nn.sigmoid(hdn)
        return x8 + jnp.dot(hdn.astype(bf16), w2[...], preferred_element_type=f32)

    w_cp(0).wait()
    x = xs[...].astype(f32)
    x0 = jnp.broadcast_to(x[0:1], (8, D))
    x1 = jnp.broadcast_to(x[1:2], (8, D))
    w_cp(1).wait()
    make_q(x0, 0)
    make_q(x1, 1)
    w_cp(2).wait()

    for j in range(wqt.shape[0]):
        wqt[j] = wq[:, j * Dh:(j + 1) * Dh].astype(wqt.dtype)
    for j in range(wot.shape[0]):
        wot[j] = wo[:, j * Dh:(j + 1) * Dh].astype(wot.dtype)

    x0 = lax.fori_loop(0, H, lambda h, a: a + attn_head(0, 0, h, True), x0)
    w_cp(3).wait()
    w_cp(4).wait()
    x0 = ffn(x0)
    make_q(x0, 0)
    for j in range(w1t.shape[0]):
        w = w1[:, j * Dh:(j + 1) * Dh]
        w1t[j] = w
        cs1[j] = jnp.broadcast_to(jnp.sum(w.astype(f32), axis=0, keepdims=True), (8, Dh))
    for j in range(w2t.shape[0]):
        w2t[j] = w2[:, j * Dh:(j + 1) * Dh]

    def colsum_q(h, c):
        cs = jnp.zeros((8, Dh), f32)
        for j in range(_REP):
            t = jnp.sum(wqt[h * _REP + j].astype(f32), axis=0, keepdims=True)
            cs = jnp.where(row % _REP == j, t, cs)
        csq[h] = cs
        return c

    lax.fori_loop(0, H, colsum_q, 0)

    x0 = lax.fori_loop(0, H, lambda h, a: a + attn_head(0, 0, h, False), x0)
    x0 = ffn(x0)
    o_ref[0:1, :] = x0[0:1].astype(o_ref.dtype)

    x1 = lax.fori_loop(
        0, H - 2, lambda h, a: a + attn_head(1, 1, h, True, transpose=True), x1)
    pls = []
    for i in (2, 1):
        kv_cp(0, G - i).wait()
        transpose_k(H - i)
        pls.append(softmax_num(qk(qs[1, H - i], 1, H - i)))
    kv_cp(1, G - 2).wait()
    p, l = pls[0]
    x1 = x1 + out_proj(jnp.dot(p, vb[1, H - 2], preferred_element_type=f32) / l, H - 2)
    h = H - 1
    p, l = pls[1]
    o8 = jnp.zeros((8, Dh), f32)
    for i, (r0, n) in enumerate(_LAST):
        vl_cp(i).wait()
        o8 = o8 + jnp.dot(p[:, r0:r0 + n], vb[1, h, r0:r0 + n, :],
                          preferred_element_type=f32)
    x1 = x1 + out_proj(o8 / l, h)

    true = (pltpu.bitcast(x1[:, :Dh], jnp.int32) | 1) != 0

    def after(val, dep):
        return val if dep is None else jnp.where(true, val, dep)

    def col(v):
        return jnp.broadcast_to(v, (Dh, Dh)).T

    def vpu_rows(acc, w_ref, tiles, row0, c_ref, c0, dep):
        cl = after(c_ref[c0:c0 + 8, :], dep)
        ch = after(c_ref[c0 + 8:c0 + 16, :], dep)
        for j, t in enumerate(tiles):
            w = w_ref[t, row0:row0 + 16, :].astype(f32)
            u = w[:8] * cl + w[8:] * ch
            acc[j] = u if acc[j] is None else acc[j] + u

    def ld(ref32, idx, r0, n):
        return pltpu.bitcast(ref32[idx + (slice(r0 // 2, (r0 + n) // 2),)], bf16)

    def ln_parts(x8):
        xb = x8.astype(bf16)
        xr = xb.astype(f32)
        for i in range(D // Dh):
            ycol[i * Dh:(i + 1) * Dh, :] = col(xr[0:1, i * Dh:(i + 1) * Dh])
        m = jnp.mean(xr, axis=-1, keepdims=True)
        d = xr - m
        v = jnp.mean(d * d, axis=-1, keepdims=True)
        return xb, m, 1.0 / jnp.sqrt(v + 1e-5)

    w1t32, w2t32 = w1t.bitcast(jnp.uint32), w2t.bitcast(jnp.uint32)
    NF = w1t.shape[0]
    NV = _NV
    NM = NF - NV

    def gated(n, deps):
        deps = [None] * _LEAD + deps[:len(deps) - _TRAIL]
        return [deps[i * len(deps) // n] for i in range(n)]

    def ffn_tail(x8):
        xb, m, r = ln_parts(x8)

        def act(u, n):
            z = (u - m * cs1[n]) * r
            return z * jax.nn.sigmoid(z)

        us = [jnp.dot(xb, ld(w1t32, (n,), 0, D), preferred_element_type=f32)
              for n in range(NM)]
        hs = [act(u, n) for n, u in enumerate(us)]
        for n in range(NV):
            hcol[n * Dh:(n + 1) * Dh, :] = col(hs[n][0:1])
        acc = [None] * NV
        for i, dep in enumerate(gated(D // 16, us)):
            vpu_rows(acc, w1t, range(NM, NF), i * 16, ycol, i * 16, dep)
        hs += [act(jnp.sum(a, axis=0, keepdims=True), NM + j)
               for j, a in enumerate(acc)]
        ds = []
        for k in range(NV, NF):
            w = jnp.concatenate([ld(w2t32, (n,), k * Dh, Dh) for n in range(D // Dh)],
                                axis=1)
            ds.append(jnp.dot(hs[k].astype(bf16), w, preferred_element_type=f32))
        acc = [None] * (D // Dh)
        for i, dep in enumerate(gated(NV * Dh // 16, [d[:, :Dh] for d in ds])):
            vpu_rows(acc, w2t, range(D // Dh), i * 16, hcol, i * 16, dep)
        out = x8 + jnp.concatenate(
            [jnp.sum(a, axis=0, keepdims=True) for a in acc], axis=1)
        for d in ds:
            out = out + d
        return out

    x1 = ffn_tail(x1)
    xb, m2, r2 = ln_parts(x1)
    r2 = r2 * (scale * 1.4426950408889634)
    q0 = jnp.dot(xb, wq[:, :_REP * Dh], preferred_element_type=f32)
    q8 = jnp.zeros((8, Dh), f32)
    for j in range(_REP):
        q8 = jnp.where(row % _REP == j, q0[:, j * Dh:(j + 1) * Dh], q8)
    qrow = {0: (q8 - m2 * csq[0]) * r2}

    vb32 = vb.bitcast(jnp.uint32)
    kt32 = kt.bitcast(jnp.uint32)
    NT = S // Dh
    oacc = [None] * (D // Dh)

    def fold4(a):
        def mix(u, v, sh):
            m = (row & sh) == 0
            return jnp.where(m, u, v) + pltpu.roll(jnp.where(m, v, u), sh, 0)
        c = mix(mix(a[0], a[1], 1), mix(a[2], a[3], 1), 2)
        return c + pltpu.roll(c, 4, 0)

    def wq_work(h):
        acc = [None] * _REP

        def chunk(r, dep):
            vpu_rows(acc, wqt, range(h * _REP, (h + 1) * _REP), r * 16, ycol, r * 16, dep)
            if r == D // 16 - 1:
                qrow[h] = (fold4(acc) - m2 * csq[h]) * r2
                for j in range(_REP):
                    qcol[h, j * Dh:(j + 1) * Dh, :] = col(qrow[h][j:j + 1])
        return [functools.partial(chunk, r) for r in range(D // 16)]

    def wo_work(h):
        def chunk(r, dep):
            vpu_rows(oacc, wot, range(D // Dh), h * _REP * Dh + r * 16,
                     ocol.at[h % 2], r * 16, dep)
        return [functools.partial(chunk, r) for r in range(_REP * Dh // 16)]

    def qk_work(h, out):
        work = []
        for t0 in range(0, _NKV, 4):
            acc = [[None] * _REP for _ in range(4)]

            def chunk(g, dep, t0=t0, acc=acc):
                qv = [after(qcol[h, j * Dh + g * 8:j * Dh + g * 8 + 8, :], dep)
                      for j in range(_REP)]
                for t in range(4):
                    kv = ktf[h, t0 + t, g * 8:g * 8 + 8, :]
                    for j in range(_REP):
                        u = kv * qv[j]
                        acc[t][j] = u if g == 0 else acc[t][j] + u
                if g == Dh // 8 - 1:
                    out.extend(fold4(a) for a in acc)
            work += [functools.partial(chunk, g) for g in range(Dh // 8)]
        return work

    def run(steps, work):
        res = []
        for i, step in enumerate(steps):
            res.append(step())
            for w in work[i * len(work) // len(steps):(i + 1) * len(work) // len(steps)]:
                w(res[i - 1][:, :Dh] if i else None)
        return res

    def qk_stage(h):
        qb = qrow[h].astype(bf16)

        def step(t0):
            kk = jnp.concatenate([ld(kt32, (h, t0 + t), 0, Dh) for t in range(4)], axis=1)
            return jnp.dot(qb, kk, preferred_element_type=f32)
        extra = []
        work = qk_work(h, extra) if h else wq_work(1) + wq_work(2)
        ss = run([functools.partial(step, t0)
                  for t0 in range(0, NT - (_NKV if h else 0), 4)], work)
        ts = [s[:, t * Dh:(t + 1) * Dh] for s in ss for t in range(4)] + extra
        return jnp.concatenate([jnp.where(row < _REP, a, b)
                                for a, b in zip(ts[0::2], ts[1::2])], axis=1)

    def pv_stage(h, s):
        m = jnp.max(s, axis=-1, keepdims=True)
        m = jnp.broadcast_to(m, (8, Dh))
        m = jnp.maximum(m, pltpu.roll(m, _REP, 0))
        p = jnp.exp2(s - jnp.tile(m, (1, NT // 2)))
        l = jnp.broadcast_to(jnp.sum(p, axis=-1, keepdims=True), (8, Dh))
        l = l + pltpu.roll(l, _REP, 0)
        p = p.astype(bf16)

        def step(i):
            g, odd = i // 2, i % 2
            vv = jnp.concatenate([ld(vb32, (1, h), (8 * g + 2 * t + odd) * Dh, Dh)
                                  for t in range(4)], axis=0)
            return jnp.dot(p[:, 4 * g * Dh:4 * (g + 1) * Dh], vv, preferred_element_type=f32)
        work = (wq_work(h + 3) if h + 3 < H else []) + (wo_work(h - 1) if h else [])
        ds = run([functools.partial(step, i) for i in range(NT // 4)], work)
        ev, od = (functools.reduce(lambda a, b: a + b, ds[i::2]) for i in range(2))
        o8 = (ev + pltpu.roll(od, _REP, 0)) / l
        if h + 1 < H:
            for j in range(_REP):
                ocol[h % 2, j * Dh:(j + 1) * Dh, :] = col(o8[j:j + 1])
        return o8

    s_prev = qk_stage(0)
    for h in range(H):
        if h + 1 < H:
            s_next = qk_stage(h + 1)
        o8 = pv_stage(h, s_prev)
        s_prev = s_next
    x1 = x1 + out_proj(o8, H - 1) + jnp.concatenate(
        [jnp.sum(a, axis=0, keepdims=True) for a in oacc], axis=1)
    x1 = ffn_tail(x1)
    o_ref[1:2, :] = x1[0:1].astype(o_ref.dtype)


@jax.jit
def pallas_interleave_layers__gqa_block_cached__dense_activation_silu__decode_kernel(
    A_x: jax.Array,
    A_k_cache: jax.Array,
    A_v_cache: jax.Array,
    A_wq: jax.Array,
    A_wo: jax.Array,
    B_x: jax.Array,
    B_w1: jax.Array,
    B_w2: jax.Array,
):
    del B_x
    B, Sq, D = A_x.shape
    _, H, S, Dh = A_k_cache.shape
    F = B_w1.shape[1]
    dt = A_k_cache.dtype
    out = pl.pallas_call(
        _kernel,
        out_shape=jax.ShapeDtypeStruct((B, D), A_x.dtype),
        in_specs=[pl.BlockSpec(memory_space=pl.ANY)] * 7,
        out_specs=pl.BlockSpec(memory_space=pltpu.VMEM),
        scratch_shapes=[
            pltpu.VMEM((B, D), A_x.dtype),
            pltpu.VMEM((B, H, S, Dh), dt),
            pltpu.VMEM((B, H, S, Dh), dt),
            pltpu.VMEM((H, S // Dh, Dh, Dh), dt),
            pltpu.VMEM(A_wq.shape, A_wq.dtype),
            pltpu.VMEM(A_wo.shape, A_wo.dtype),
            pltpu.VMEM(B_w1.shape, B_w1.dtype),
            pltpu.VMEM(B_w2.shape, B_w2.dtype),
            pltpu.VMEM((A_wq.shape[1] // Dh, D, Dh), jnp.float32),
            pltpu.VMEM((D // Dh, A_wo.shape[0], Dh), jnp.float32),
            pltpu.VMEM((F // Dh, D, Dh), B_w1.dtype),
            pltpu.VMEM((D // Dh, F, Dh), B_w2.dtype),
            pltpu.VMEM((D, Dh), jnp.float32),
            pltpu.VMEM((2, _REP * Dh, Dh), jnp.float32),
            pltpu.VMEM((_NV * Dh, Dh), jnp.float32),
            pltpu.VMEM((F // Dh, 8, Dh), jnp.float32),
            pltpu.VMEM((H, 8, Dh), jnp.float32),
            pltpu.VMEM((H, _NKV, Dh, Dh), jnp.float32),
            pltpu.VMEM((H, _REP * Dh, Dh), jnp.float32),
            pltpu.VMEM((B, H, 8, Dh), jnp.float32),
            pltpu.SemaphoreType.DMA((len(_GROUPS),)),
            pltpu.SemaphoreType.DMA((len(_GROUPS) - 1,)),
            pltpu.SemaphoreType.DMA((5,)),
            pltpu.SemaphoreType.DMA((len(_LAST),)),
        ],
        compiler_params=pltpu.CompilerParams(vmem_limit_bytes=126 * 1024 * 1024),
    )(A_x.reshape(B, D), A_k_cache, A_v_cache, A_wq, A_wo, B_w1, B_w2)
    return out.reshape(B, Sq, D)
```

```python
import functools

import jax
import jax.numpy as jnp
from jax import lax
import jax.experimental.pallas as pl
import jax.experimental.pallas.tpu as pltpu


_NKV = 4
_NV = 3
_LEAD, _TRAIL = 2, 5
_REP = 4
_GROUPS = ((0, 0, 8), (1, 0, 4), (1, 4, 2), (1, 6, 1), (1, 7, 1))
_LAST = ((0, 4096), (4096, 2560), (6656, 1024), (7680, 512))


def _ln(x):
    m = jnp.mean(x, axis=-1, keepdims=True)
    d = x - m
    v = jnp.mean(d * d, axis=-1, keepdims=True)
    return d / jnp.sqrt(v + 1e-5)


def _kernel(x_hbm, k_hbm, v_hbm, wq_hbm, wo_hbm, w1_hbm, w2_hbm, o_ref,
            xs, kb, vb, kt, wq, wo, w1, w2, wqt, wot, w1t, w2t, ycol, ocol, hcol,
            cs1, csq, ktf, qcol, qs, ksem, vsem, wsem, lsem):
    B, H, S, Dh = vb.shape
    kbuf = {1: kb}
    D = xs.shape[-1]
    scale = Dh ** -0.5
    f32, bf16 = jnp.float32, jnp.bfloat16

    def w_cp(i):
        src, dst = ((x_hbm, xs), (wq_hbm, wq), (wo_hbm, wo), (w1_hbm, w1),
                    (w2_hbm, w2))[i]
        return pltpu.make_async_copy(src, dst, wsem.at[i])

    def kv_cp(t, g):
        b, h0, n = _GROUPS[g]
        if t == 0:
            return pltpu.make_async_copy(k_hbm.at[b, pl.ds(h0, n)],
                                         kbuf[b].at[pl.ds(h0, n)], ksem.at[g])
        return pltpu.make_async_copy(v_hbm.at[b, pl.ds(h0, n)],
                                     vb.at[b, pl.ds(h0, n)], vsem.at[g])

    def vl_cp(i):
        r0, n = _LAST[i]
        return pltpu.make_async_copy(v_hbm.at[B - 1, H - 1, pl.ds(r0, n)],
                                     vb.at[B - 1, H - 1, pl.ds(r0, n)], lsem.at[i])

    G = len(_GROUPS)

    def kv_wait(t, b, h):
        for g, (gb, h0, _) in enumerate(_GROUPS[:-2]):
            if gb == b:
                pl.when(h == h0)(kv_cp(t, g).wait)

    row = lax.broadcasted_iota(jnp.int32, (8, Dh), 0)

    def make_q(x8, slot):
        q = jnp.dot(_ln(x8).astype(bf16), wq[...], preferred_element_type=f32)
        for h in range(H):
            qh = jnp.zeros((8, Dh), f32)
            for j in range(_REP):
                c = (h * _REP + j) * Dh
                qh = jnp.where(row == j, q[:, c:c + Dh], qh)
            qs[slot, h] = qh

    def softmax_num(s):
        s = s * scale
        m = jnp.max(s, axis=-1, keepdims=True)
        p = jnp.exp(s - m)
        return p.astype(bf16), jnp.sum(p, axis=-1, keepdims=True)

    def qk(q8, b, h):
        return lax.dot_general(q8.astype(bf16), kbuf[b][h], (((1,), (1,)), ((), ())),
                               preferred_element_type=f32)

    def out_proj(o8, h):
        o = jnp.concatenate(
            [jnp.broadcast_to(o8[j:j + 1], (8, Dh)) for j in range(_REP)], axis=1)
        r0 = h * _REP * Dh
        w = wo[pl.ds(r0 if isinstance(h, int) else pl.multiple_of(r0, _REP * Dh), _REP * Dh), :]
        return jnp.dot(o.astype(bf16), w, preferred_element_type=f32)

    def transpose_k(h):
        for t in range(S // Dh):
            tile = kb[h, t * Dh:(t + 1) * Dh, :].T
            kt[h, t] = pltpu.bitcast(tile, jnp.uint32)
            if t >= S // Dh - _NKV:
                ktf[h, t - (S // Dh - _NKV)] = tile.astype(f32)

    def attn_head(slot, b, h, wait, transpose=False):
        if wait:
            kv_wait(0, b, h)
        if transpose:
            transpose_k(h)
        p, l = softmax_num(qk(qs[slot, h], b, h))
        if wait:
            kv_wait(1, b, h)
        o8 = jnp.dot(p, vb[b, h], preferred_element_type=f32) / l
        return out_proj(o8, h)

    def ffn(x8):
        hdn = jnp.dot(_ln(x8).astype(bf16), w1[...], preferred_element_type=f32)
        hdn = hdn * jax.nn.sigmoid(hdn)
        return x8 + jnp.dot(hdn.astype(bf16), w2[...], preferred_element_type=f32)

    def batch0(kb0):
        kbuf[0] = kb0
        w_cp(1).start()
        queue = [w_cp(i) for i in (0, 2, 3, 4)]
        for g in range(G - 2):
            queue += [kv_cp(0, g), kv_cp(1, g)]
        queue += [kv_cp(0, G - 2), kv_cp(0, G - 1), kv_cp(1, G - 2)]
        queue += [vl_cp(i) for i in range(len(_LAST))]

        def enqueue(i, c):
            for j, cp in enumerate(queue):
                pl.when(i == j)(cp.start)
            return c

        lax.fori_loop(0, len(queue), enqueue, 0)

        w_cp(0).wait()
        x = xs[...].astype(f32)
        x0 = jnp.broadcast_to(x[0:1], (8, D))
        x1 = jnp.broadcast_to(x[1:2], (8, D))
        w_cp(1).wait()
        make_q(x0, 0)
        make_q(x1, 1)
        w_cp(2).wait()

        for j in range(wqt.shape[0]):
            wqt[j] = wq[:, j * Dh:(j + 1) * Dh].astype(wqt.dtype)
        for j in range(wot.shape[0]):
            wot[j] = wo[:, j * Dh:(j + 1) * Dh].astype(wot.dtype)

        x0 = lax.fori_loop(0, H, lambda h, a: a + attn_head(0, 0, h, True), x0)
        w_cp(3).wait()
        w_cp(4).wait()
        x0 = ffn(x0)
        make_q(x0, 0)
        for j in range(w1t.shape[0]):
            w = w1[:, j * Dh:(j + 1) * Dh]
            w1t[j] = pltpu.bitcast(w, jnp.uint32)
            cs1[j] = jnp.broadcast_to(jnp.sum(w.astype(f32), axis=0, keepdims=True), (8, Dh))
        for j in range(w2t.shape[0]):
            w2t[j] = pltpu.bitcast(w2[:, j * Dh:(j + 1) * Dh], jnp.uint32)

        def colsum_q(h, c):
            cs = jnp.zeros((8, Dh), f32)
            for j in range(_REP):
                t = jnp.sum(wqt[h * _REP + j].astype(f32), axis=0, keepdims=True)
                cs = jnp.where(row % _REP == j, t, cs)
            csq[h] = cs
            return c

        lax.fori_loop(0, H, colsum_q, 0)

        x0 = lax.fori_loop(0, H, lambda h, a: a + attn_head(0, 0, h, False), x0)
        x0 = ffn(x0)
        return x0, x1

    x0, x1 = pl.run_scoped(batch0, pltpu.VMEM((H, S, Dh), kb.dtype))

    def batch1(vt, x1):
        def pack_v(h, r0, n):
            vt[h, r0 // 2:(r0 + n) // 2, :] = pltpu.bitcast(vb[1, h, pl.ds(r0, n), :], jnp.uint32)

        def head1(h, a):
            a = a + attn_head(1, 1, h, True, transpose=True)
            pack_v(h, 0, S)
            return a

        x1 = lax.fori_loop(
            0, H - 2, lambda h, a: head1(h, a), x1)
        pls = []
        for i in (2, 1):
            kv_cp(0, G - i).wait()
            transpose_k(H - i)
            pls.append(softmax_num(qk(qs[1, H - i], 1, H - i)))
        kv_cp(1, G - 2).wait()
        pack_v(H - 2, 0, S)
        p, l = pls[0]
        x1 = x1 + out_proj(jnp.dot(p, vb[1, H - 2], preferred_element_type=f32) / l, H - 2)
        h = H - 1
        p, l = pls[1]
        o8 = jnp.zeros((8, Dh), f32)
        for i, (r0, n) in enumerate(_LAST):
            vl_cp(i).wait()
            pack_v(h, r0, n)
            o8 = o8 + jnp.dot(p[:, r0:r0 + n], vb[1, h, r0:r0 + n, :],
                              preferred_element_type=f32)
        x1 = x1 + out_proj(o8 / l, h)

        true = (pltpu.bitcast(x1[:, :Dh], jnp.int32) | 1) != 0

        def after(val, dep):
            return val if dep is None else jnp.where(true, val, dep)

        def col(v):
            return jnp.broadcast_to(v, (Dh, Dh)).T

        def vpu_rows(acc, w_ref, tiles, row0, c_ref, c0, dep):
            cl = after(c_ref[c0:c0 + 8, :], dep)
            ch = after(c_ref[c0 + 8:c0 + 16, :], dep)
            for j, t in enumerate(tiles):
                if w_ref.dtype == jnp.uint32:
                    w = ld(w_ref, (t,), row0, 16).astype(f32)
                else:
                    w = w_ref[t, row0:row0 + 16, :]
                u = w[:8] * cl + w[8:] * ch
                acc[j] = u if acc[j] is None else acc[j] + u

        def ld(ref32, idx, r0, n):
            return pltpu.bitcast(ref32[idx + (slice(r0 // 2, (r0 + n) // 2),)], bf16)

        def ln_parts(x8):
            xb = x8.astype(bf16)
            xr = xb.astype(f32)
            for i in range(D // Dh):
                ycol[i * Dh:(i + 1) * Dh, :] = col(xr[0:1, i * Dh:(i + 1) * Dh])
            m = jnp.mean(xr, axis=-1, keepdims=True)
            d = xr - m
            v = jnp.mean(d * d, axis=-1, keepdims=True)
            return xb, m, 1.0 / jnp.sqrt(v + 1e-5)

        NF = w1t.shape[0]
        NV = _NV
        NM = NF - NV

        def gated(n, deps):
            deps = [None] * _LEAD + deps[:len(deps) - _TRAIL]
            return [deps[i * len(deps) // n] for i in range(n)]

        def ffn_tail(x8):
            xb, m, r = ln_parts(x8)

            def act(u, n):
                z = (u - m * cs1[n]) * r
                return z * jax.nn.sigmoid(z)

            us = [jnp.dot(xb, ld(w1t, (n,), 0, D), preferred_element_type=f32)
                  for n in range(NM)]
            hs = [act(u, n) for n, u in enumerate(us)]
            for n in range(NV):
                hcol[n * Dh:(n + 1) * Dh, :] = col(hs[n][0:1])
            acc = [None] * NV
            for i, dep in enumerate(gated(D // 16, us)):
                vpu_rows(acc, w1t, range(NM, NF), i * 16, ycol, i * 16, dep)
            hs += [act(jnp.sum(a, axis=0, keepdims=True), NM + j)
                   for j, a in enumerate(acc)]
            ds = []
            for k in range(NV, NF):
                w = jnp.concatenate([ld(w2t, (n,), k * Dh, Dh) for n in range(D // Dh)],
                                    axis=1)
                ds.append(jnp.dot(hs[k].astype(bf16), w, preferred_element_type=f32))
            acc = [None] * (D // Dh)
            for i, dep in enumerate(gated(NV * Dh // 16, [d[:, :Dh] for d in ds])):
                vpu_rows(acc, w2t, range(D // Dh), i * 16, hcol, i * 16, dep)
            out = x8 + jnp.concatenate(
                [jnp.sum(a, axis=0, keepdims=True) for a in acc], axis=1)
            for d in ds:
                out = out + d
            return out

        x1 = ffn_tail(x1)
        xb, m2, r2 = ln_parts(x1)
        r2 = r2 * (scale * 1.4426950408889634)
        q0 = jnp.dot(xb, wq[:, :_REP * Dh], preferred_element_type=f32)
        q8 = jnp.zeros((8, Dh), f32)
        for j in range(_REP):
            q8 = jnp.where(row % _REP == j, q0[:, j * Dh:(j + 1) * Dh], q8)
        qrow = {0: (q8 - m2 * csq[0]) * r2}

        NT = S // Dh
        oacc = [None] * (D // Dh)

        def fold4(a):
            def mix(u, v, sh):
                m = (row & sh) == 0
                return jnp.where(m, u, v) + pltpu.roll(jnp.where(m, v, u), sh, 0)
            c = mix(mix(a[0], a[1], 1), mix(a[2], a[3], 1), 2)
            return c + pltpu.roll(c, 4, 0)

        def wq_work(h):
            acc = [None] * _REP

            def chunk(r, dep):
                vpu_rows(acc, wqt, range(h * _REP, (h + 1) * _REP), r * 16, ycol, r * 16, dep)
                if r == D // 16 - 1:
                    qrow[h] = (fold4(acc) - m2 * csq[h]) * r2
                    for j in range(_REP):
                        qcol[h, j * Dh:(j + 1) * Dh, :] = col(qrow[h][j:j + 1])
            return [functools.partial(chunk, r) for r in range(D // 16)]

        def wo_work(h):
            def chunk(r, dep):
                vpu_rows(oacc, wot, range(D // Dh), h * _REP * Dh + r * 16,
                         ocol.at[h % 2], r * 16, dep)
            return [functools.partial(chunk, r) for r in range(_REP * Dh // 16)]

        def qk_work(h, out):
            work = []
            for t0 in range(0, _NKV, 4):
                acc = [[None] * _REP for _ in range(4)]

                def chunk(g, dep, t0=t0, acc=acc):
                    qv = [after(qcol[h, j * Dh + g * 8:j * Dh + g * 8 + 8, :], dep)
                          for j in range(_REP)]
                    for t in range(4):
                        kv = ktf[h, t0 + t, g * 8:g * 8 + 8, :]
                        for j in range(_REP):
                            u = kv * qv[j]
                            acc[t][j] = u if g == 0 else acc[t][j] + u
                    if g == Dh // 8 - 1:
                        out.extend(fold4(a) for a in acc)
                work += [functools.partial(chunk, g) for g in range(Dh // 8)]
            return work

        def run(steps, work):
            res = []
            for i, step in enumerate(steps):
                res.append(step())
                for w in work[i * len(work) // len(steps):(i + 1) * len(work) // len(steps)]:
                    w(res[i - 1][:, :Dh] if i else None)
            return res

        def qk_stage(h):
            qb = qrow[h].astype(bf16)

            def step(t0):
                kk = jnp.concatenate([ld(kt, (h, t0 + t), 0, Dh) for t in range(4)], axis=1)
                return jnp.dot(qb, kk, preferred_element_type=f32)
            extra = []
            work = qk_work(h, extra) if h else wq_work(1) + wq_work(2)
            ss = run([functools.partial(step, t0)
                      for t0 in range(0, NT - (_NKV if h else 0), 4)], work)
            ts = [s[:, t * Dh:(t + 1) * Dh] for s in ss for t in range(4)] + extra
            return jnp.concatenate([jnp.where(row < _REP, a, b)
                                    for a, b in zip(ts[0::2], ts[1::2])], axis=1)

        def pv_stage(h, s):
            m = jnp.max(s, axis=-1, keepdims=True)
            m = jnp.broadcast_to(m, (8, Dh))
            m = jnp.maximum(m, pltpu.roll(m, _REP, 0))
            p = jnp.exp2(s - jnp.tile(m, (1, NT // 2)))
            l = jnp.broadcast_to(jnp.sum(p, axis=-1, keepdims=True), (8, Dh))
            l = l + pltpu.roll(l, _REP, 0)
            p = p.astype(bf16)

            def step(i):
                g, odd = i // 2, i % 2
                vv = jnp.concatenate([ld(vt, (h,), (8 * g + 2 * t + odd) * Dh, Dh)
                                      for t in range(4)], axis=0)
                return jnp.dot(p[:, 4 * g * Dh:4 * (g + 1) * Dh], vv, preferred_element_type=f32)
            work = (wq_work(h + 3) if h + 3 < H else []) + (wo_work(h - 1) if h else [])
            ds = run([functools.partial(step, i) for i in range(NT // 4)], work)
            ev, od = (functools.reduce(lambda a, b: a + b, ds[i::2]) for i in range(2))
            o8 = (ev + pltpu.roll(od, _REP, 0)) / l
            if h + 1 < H:
                for j in range(_REP):
                    ocol[h % 2, j * Dh:(j + 1) * Dh, :] = col(o8[j:j + 1])
            return o8

        s_prev = qk_stage(0)
        for h in range(H):
            if h + 1 < H:
                s_next = qk_stage(h + 1)
            o8 = pv_stage(h, s_prev)
            s_prev = s_next
        x1 = x1 + out_proj(o8, H - 1) + jnp.concatenate(
            [jnp.sum(a, axis=0, keepdims=True) for a in oacc], axis=1)
        x1 = ffn_tail(x1)
        first = lax.broadcasted_iota(jnp.int32, (8, D), 0) == 0
        o_ref[...] = jnp.where(first, x0, x1)[:B].astype(o_ref.dtype)

    pl.run_scoped(functools.partial(batch1, x1=x1),
                  pltpu.VMEM((H, S // 2, Dh), jnp.uint32))


@jax.jit
def pallas_interleave_layers__gqa_block_cached__dense_activation_silu__decode_kernel(
    A_x: jax.Array,
    A_k_cache: jax.Array,
    A_v_cache: jax.Array,
    A_wq: jax.Array,
    A_wo: jax.Array,
    B_x: jax.Array,
    B_w1: jax.Array,
    B_w2: jax.Array,
):
    del B_x
    B, Sq, D = A_x.shape
    _, H, S, Dh = A_k_cache.shape
    F = B_w1.shape[1]
    dt = A_k_cache.dtype
    out = pl.pallas_call(
        _kernel,
        out_shape=jax.ShapeDtypeStruct((B, D), A_x.dtype),
        in_specs=[pl.BlockSpec(memory_space=pl.ANY)] * 7,
        out_specs=pl.BlockSpec(memory_space=pltpu.VMEM),
        scratch_shapes=[
            pltpu.VMEM((B, D), A_x.dtype),
            pltpu.VMEM((H, S, Dh), dt),
            pltpu.VMEM((B, H, S, Dh), dt),
            pltpu.VMEM((H, S // Dh, Dh // 2, Dh), jnp.uint32),
            pltpu.VMEM(A_wq.shape, A_wq.dtype),
            pltpu.VMEM(A_wo.shape, A_wo.dtype),
            pltpu.VMEM(B_w1.shape, B_w1.dtype),
            pltpu.VMEM(B_w2.shape, B_w2.dtype),
            pltpu.VMEM((A_wq.shape[1] // Dh, D, Dh), jnp.float32),
            pltpu.VMEM((D // Dh, A_wo.shape[0], Dh), jnp.float32),
            pltpu.VMEM((F // Dh, D // 2, Dh), jnp.uint32),
            pltpu.VMEM((D // Dh, F // 2, Dh), jnp.uint32),
            pltpu.VMEM((D, Dh), jnp.float32),
            pltpu.VMEM((2, _REP * Dh, Dh), jnp.float32),
            pltpu.VMEM((_NV * Dh, Dh), jnp.float32),
            pltpu.VMEM((F // Dh, 8, Dh), jnp.float32),
            pltpu.VMEM((H, 8, Dh), jnp.float32),
            pltpu.VMEM((H, _NKV, Dh, Dh), jnp.float32),
            pltpu.VMEM((H, _REP * Dh, Dh), jnp.float32),
            pltpu.VMEM((B, H, 8, Dh), jnp.float32),
            pltpu.SemaphoreType.DMA((len(_GROUPS),)),
            pltpu.SemaphoreType.DMA((len(_GROUPS) - 1,)),
            pltpu.SemaphoreType.DMA((5,)),
            pltpu.SemaphoreType.DMA((len(_LAST),)),
        ],
        compiler_params=pltpu.CompilerParams(vmem_limit_bytes=126 * 1024 * 1024),
    )(A_x.reshape(B, D), A_k_cache, A_v_cache, A_wq, A_wo, B_w1, B_w2)
    return out.reshape(B, Sq, D)
```
